```python
import os as _os
_os.environ.setdefault("JAX_PLATFORMS", "cpu")
import jax
import jax.numpy as jnp

def _softmax(x, axis=-1):
    return jax.nn.softmax(x, axis=axis)
def _gelu(x):
    return jax.nn.gelu(x, approximate=True)
def _silu(x):
    return jax.nn.silu(x)
def _sigmoid(x):
    return jax.nn.sigmoid(x)
def _layernorm(x, axis=-1, eps=1e-5):
    m = jnp.mean(x, axis=axis, keepdims=True)
    v = jnp.var(x, axis=axis, keepdims=True)
    return (x - m) / jnp.sqrt(v + eps)
def _scatter_add(tgt, idx, src, axis=0):
    return tgt.at[idx].add(src)
def _segment_sum(src, seg, n):
    return jax.ops.segment_sum(src, seg, n)
class _Rng:
    def __init__(self, key):
        self._k = key
    def _next(self):
        self._k, sub = jax.random.split(self._k)
        return sub
    def normal(self, shape):
        return jax.random.normal(self._next(), shape, dtype=jnp.bfloat16)
    def randint(self, lo, hi, shape):
        return jax.random.randint(self._next(), shape, lo, hi, dtype=jnp.int32)
    def uniform(self, shape, lo=0.0, hi=1.0):
        return jax.random.uniform(self._next(), shape, jnp.bfloat16, lo, hi)
    def permutation(self, n):
        return jax.random.permutation(self._next(), n)


kernel_name = 'concat_heads__linear_attn_block__sliding_local_dilated__prompt'

def setup_inputs():
    _rng = _Rng(jax.random.key(int.from_bytes(__import__("os").urandom(4), "little")))
    _w = (lambda a: (lambda t: t.astype(jnp.bfloat16) if jnp.issubdtype(t.dtype, jnp.floating) else t)(jnp.asarray(a)))
    def _A_setup():
        B, S, D = 1, 2048, 576
        return {
            "x": _w((lambda *s: _rng.normal(s) * 0.05)(B, S, D)),
            "wqkv": _w((lambda *s: _rng.normal(s) * 1.6)(D, 3 * D)),
            "wo": _w((lambda *s: _rng.normal(s) * 0.4)(D, D)),
        }
    _A_in = _A_setup()

    def _B_setup():
        B, S, D = 1, 2048, 576
        return {
            "x": _w((lambda *s: _rng.normal(s) * 0.2)(B, S, D)),
            "wqkv": _w((lambda *s: _rng.normal(s) * 0.2)(D, 3 * D)),
            "wo": _w((lambda *s: _rng.normal(s) * 0.05)(D, D)),
        }
    _B_in = _B_setup()

    return {
        "A_x": _A_in["x"],
        "A_wqkv": _A_in["wqkv"],
        "A_wo": _A_in["wo"],
        "B_x": _B_in["x"],
        "B_wqkv": _B_in["wqkv"],
        "B_wo": _B_in["wo"],
    }

def reference(A_x, A_wqkv, A_wo, B_x, B_wqkv, B_wo):
    def _A_ref(x, wqkv, wo):
        B, S, D = x.shape
        H = 32; Dh = D // H
        qkv = (lambda x, *d: x.transpose(*d))((x @ wqkv).reshape(B, S, 3, H, Dh), 2, 0, 3, 1, 4)
        q, k, v = qkv[0], qkv[1], qkv[2]
        phi = lambda t: jnp.where(t > 0, t + 1, jnp.exp(t)) + 1e-6
        pq, pk = phi(q), phi(k)
        kv = jnp.einsum("bhsd,bhse->bhde", pk, v)
        z = jnp.einsum("bhsd->bhd", pk)
        num = jnp.einsum("bhqd,bhde->bhqe", pq, kv)
        den = jnp.einsum("bhqd,bhd->bhq", pq, z)[..., None] + 1e-6
        o = num / den
        return (lambda x, *d: x.transpose(*d))(o, 0, 2, 1, 3).reshape(B, S, D) @ wo

    def _B_ref(x, wqkv, wo):
        B, S, D = x.shape
        H = 32; Dh = D // H
        W, dil = 8, 2
        qkv = (lambda x, *d: x.transpose(*d))((x @ wqkv).reshape(B, S, 3, H, Dh), 2, 0, 3, 1, 4)
        q, k, v = qkv[0], qkv[1], qkv[2]
        scale = Dh ** -0.5
        pos = jnp.arange(S)
        off = jnp.arange(W) * dil
        idx = pos[:, None] - off[None, :]
        mask = idx >= 0
        idx_c = jnp.where(mask, idx, 0).reshape(-1)
        kg = k[:, :, idx_c, :].reshape(B, H, S, W, Dh)
        vg = v[:, :, idx_c, :].reshape(B, H, S, W, Dh)
        logits = jnp.einsum("bhsd,bhswd->bhsw", q, kg) * scale
        logits = jnp.where(mask[None, None, :, :], logits, -1e9)
        attn = _softmax(logits, axis=-1)
        o = jnp.einsum("bhsw,bhswd->bhsd", attn, vg)
        return (lambda x, *d: x.transpose(*d))(o, 0, 2, 1, 3).reshape(B, S, D) @ wo

    a = _A_ref(A_x, A_wqkv, A_wo)
    b = _B_ref(B_x, B_wqkv, B_wo)
    return jnp.concatenate([a, b], axis=-1)
```

```python
import functools
import math

import jax
import jax.numpy as jnp
from jax import lax
import jax.experimental.pallas as pl
import jax.experimental.pallas.tpu as pltpu

S = 2048
D = 576
H = 32
DH = 18
W = 8
DIL = 2
HALO = 24
DP = 640
NB_T = 12
NXY = 192

F32 = jnp.float32
BF16 = jnp.bfloat16
U32 = jnp.uint32
NT = (((1,), (1,)), ((), ()))

SB1 = 512
SB2 = 256
BM = 128
AM = 288
RGA = 16
RG = 16
RQ = 96
HG = 16
NXC = 4
OUT_BARRIER = 3
LOG2E = math.log2(math.e)


def _phi(t):
    return jnp.where(t > 0, t + 1.0, jnp.exp(t)) + 1e-6


def _dot_nt(a, b):
    return lax.dot_general(a, b, NT, preferred_element_type=F32)


def _dot(a, b):
    return jnp.dot(a, b, preferred_element_type=F32)


def _ld(ref, r0, nr, c0, nc):
    return pltpu.bitcast(ref[pl.ds(r0 // 2, nr // 2), pl.ds(c0, nc)], BF16)


def _st(ref, r0, c0, val):
    nr, nc = val.shape
    ref[pl.ds(r0 // 2, nr // 2), pl.ds(c0, nc)] = pltpu.bitcast(val.astype(BF16), U32)


def _b_slab_src(slab):
    if slab < 48:
        return slab // 16, slab % 16
    return (slab - 48) // 2, 16 + slab % 2


def _interleave(ms, vs, lead=0):
    for m in ms[:lead]:
        m()
    ms = ms[lead:]
    if not ms:
        for v in vs:
            v()
        return
    done = 0
    for k, m in enumerate(ms):
        m()
        tgt = (k + 1) * len(vs) // len(ms)
        while done < tgt:
            vs[done]()
            done += 1


def _kernel(xa_h, wa_h, woa_h, xb_h, wb_h, wob_h, out_h,
            xa, xb, wa_lo, wa_mid, wa_hi, woa, wb, wob,
            wkT, wqT, wbT, wobP, mT, zd,
            ts_a, ts_b, ws_b, ms, zs,
            g_acc, gt_acc, z_acc, m_acc, pkT, pqT, xbn, kraw, invs, oaT, wo4T, bdS, xyT,
            qb, kv, ob, lg, outv,
            sem_x, sem_w, sem_o):
    n1 = S // SB1
    n2 = S // SB2
    nx = NXC
    sbx = S // nx

    def cp(src, dst, sem):
        return pltpu.make_async_copy(src, dst, sem)

    xa_cp = [cp(xa_h.at[:, pl.ds(i * sbx, sbx)], xa.at[:, pl.ds(i * sbx, sbx)], sem_x.at[i]) for i in range(nx)]
    xb_cp = [cp(xb_h.at[:, pl.ds(i * sbx, sbx)], xb.at[:, pl.ds(i * sbx, sbx)], sem_x.at[nx + i]) for i in range(nx)]
    wa_mid_cp = [cp(wa_h.at[pl.ds(kt * 128, 128 if kt < 4 else 64), pl.ds(512, 640)],
                    wa_mid.at[pl.ds(kt * 128, 128 if kt < 4 else 64), :], sem_w.at[6 + kt]) for kt in range(5)]
    wa_lo_cp = cp(wa_h.at[:, pl.ds(0, 512)], wa_lo, sem_w.at[1])
    wa_hi_cp = cp(wa_h.at[:, pl.ds(1152, 576)], wa_hi, sem_w.at[2])
    wb_cp = cp(wb_h, wb, sem_w.at[3])
    woa_cp = cp(woa_h, woa, sem_w.at[4])
    wob_cp = cp(wob_h, wob, sem_w.at[5])

    lane = lax.broadcasted_iota(jnp.int32, (RG, 128), 1)

    def kw_of(kt):
        return 128 if kt < 4 else 64

    def prep_wk(kt):
        kw = kw_of(kt)
        blk = wa_mid[pl.ds(kt * 128, kw), :]
        t = blk.T
        _st(wkT, 0, kt * 128, t[64:, :])
        ts_a[kt, pl.ds(512, 64), pl.ds(0, kw)] = t[:64, :].astype(F32)

    def prep_wq_T(kt):
        kw = kw_of(kt)
        blk = wa_lo[pl.ds(kt * 128, kw), :]
        ts_a[kt, pl.ds(0, 512), pl.ds(0, kw)] = blk.astype(F32).T

    def prep_wq_perm(kt):
        kw = kw_of(kt)
        for d in range(DH):
            r = ts_a[kt, pl.ds(d, H, stride=DH), :]
            _st(wqT, d * H, kt * 128, r[:, :kw])

    def prep_wb_T(kt, c0, c1):
        kw = kw_of(kt)
        blk = wb[pl.ds(kt * 128, kw), pl.ds(c0, c1 - c0)]
        ts_b[kt, pl.ds(c0, c1 - c0), pl.ds(0, kw)] = blk.astype(F32).T

    def prep_wb_perm(kt, s0, s1):
        kw = kw_of(kt)
        for slab in range(s0, s1):
            part, d = _b_slab_src(slab)
            r = ts_b[kt, pl.ds(part * D + d, H, stride=DH), :]
            _st(wbT, slab * H, kt * 128, r[:, :kw])

    def prep_wob_shift(r0, nr):
        wf = wob[pl.ds(r0, nr), :].astype(F32)
        wpad = jnp.concatenate([jnp.zeros((nr, 64), F32), wf], axis=1)
        for t in range(5):
            ws_b[t, pl.ds(r0, nr), :] = wpad[:, t * 128:(t + 1) * 128]

    def prep_wob_perm(t):
        for d in range(DH):
            r = ws_b[t, pl.ds(d, H, stride=DH), :]
            row = d * H if d < 16 else (d + 2) * H
            _st(wobP, row, t * 128, r)

    def b_xT(j):
        _st(xbn, j * 128, 0, xb[:, pl.ds(j * 128, 128)].T)

    def a_kT(j):
        for r0 in range(0, D, AM):
            kraw[j, pl.ds(r0, AM), :] = _dot(_ld(wkT, r0, AM, 0, D), xa[:, pl.ds(j * 128, 128)])

    def a_kpost(j, r0, nr):
        pk = _phi(kraw[j, pl.ds(r0, nr), :])
        if j == 0:
            z_acc[pl.ds(r0, nr), :] = pk
        else:
            z_acc[pl.ds(r0, nr), :] += pk
        _st(pkT, r0, j * 128, pk)

    def a_G(b, n):
        nw = kw_of(n)
        if n == 4:
            g = _dot_nt(xa[pl.ds(512, 64), pl.ds(b * SB1, SB1)], _ld(pkT, 0, D, b * SB1, SB1))
            if b == 0:
                gt_acc[...] = g
            elif b < n1 - 1:
                gt_acc[...] += g
            else:
                g_acc[:, pl.ds(512, 64)] = (gt_acc[...] + g).T
            return
        g = _dot_nt(_ld(pkT, 0, D, b * SB1, SB1), xa[pl.ds(n * 128, nw), pl.ds(b * SB1, SB1)])
        if b == 0:
            g_acc[:, pl.ds(n * 128, nw)] = g
        else:
            g_acc[:, pl.ds(n * 128, nw)] += g

    def band(c):
        cw = kw_of(c)
        h_lo = (128 * c) // DH
        h_hi = (128 * c + cw - 1) // DH
        r0 = (DH * h_lo) // 16 * 16
        r1 = min(D, -(-(DH * (h_hi + 1)) // 16) * 16)
        return cw, r0, r1

    def a_prep_kv(c):
        cw, r0, r1 = band(c)
        g16 = g_acc[pl.ds(r0, r1 - r0), :].astype(BF16)
        kvf = _dot(g16, wa_hi[:, pl.ds(c * 128, cw)])
        rr = lax.broadcasted_iota(jnp.int32, (r1 - r0, cw), 0) + r0
        cc = lax.broadcasted_iota(jnp.int32, (r1 - r0, cw), 1) + c * 128
        hr = (rr * 3641) >> 16
        hc = (cc * 3641) >> 16
        _st(bdS.at[c], 0, 0, jnp.where(hr == hc, kvf, 0.0))

    def a_prep_M(c):
        cw, r0, r1 = band(c)
        mc = _dot(_ld(bdS.at[c], 0, r1 - r0, 0, cw), woa[pl.ds(c * 128, cw), :])
        if c == 0:
            m_acc[pl.ds(r0, r1 - r0), :] = mc
            m_acc[pl.ds(r1, D - r1), :] = jnp.zeros((D - r1, D), F32)
        else:
            m_acc[pl.ds(r0, r1 - r0), :] += mc

    def a_prep_z():
        z = jnp.sum(z_acc[...], axis=1, keepdims=True)
        zs[...] = jnp.broadcast_to(z, (D, 128))
        for d in range(DH):
            zd[pl.ds(d * H, H), :] = zs[pl.ds(d, H, stride=DH), :]

    def a_prep_perm(t):
        tw = kw_of(t)
        ms[t, :, pl.ds(0, tw)] = m_acc[:, pl.ds(t * 128, tw)]
        rows = [ms[t, pl.ds(d, H, stride=DH), :][:, :tw].astype(BF16) for d in range(DH)]
        md = jnp.concatenate(rows, axis=0)
        _st(mT, t * 128, 0, md.T)

    def b_proj(i, t0):
        for r0 in range(i * SB2, (i + 1) * SB2, BM):
            b_proj_rows(r0, t0)

    def b_proj_rows(r0, t0):
        xblk = _ld(xbn, r0, BM, 0, D)
        nt = 1
        r = _dot_nt(xblk, _ld(wbT, t0 * 128, nt * 128, 0, D))
        c = (DH ** -0.5) * LOG2E
        for u in range(nt):
            t = t0 + u
            val = r[:, u * 128:(u + 1) * 128]
            if t < 4:
                qb[t, pl.ds(r0, BM), :] = val * c
            else:
                kv[t - 4, pl.ds(HALO + r0, BM), :] = val

    def b_xy(j):
        xyT[j] = _dot(_ld(wbT, NB_T * 128, NXY, 0, D), xb[:, pl.ds(j * 128, 128)])

    def b_xypost(j):
        c = (DH ** -0.5) * LOG2E
        xq = jnp.concatenate([xyT[j, pl.ds(0, 64), :] * c, jnp.zeros((64, 128), F32)], axis=0)
        qb[4, pl.ds(j * 128, 128), :] = xq.T
        kv[8, pl.ds(HALO + j * 128, 128), :] = xyT[j, pl.ds(64, 128), :].T

    def b_logits(r0):
        nv = RGA // 8
        q = [qb[t, pl.ds(r0, RGA), :] for t in range(5)]
        acc = [None] * W
        for t in range(5):
            src = t if t < 4 else 8
            for c in range(4):
                kk = kv[src, pl.ds(HALO + r0 - DIL * c - 8, RGA + 8), :]
                for w, kx in ((c, kk[8:, :]), (c + 4, kk[:RGA, :])):
                    p = q[t] * kx
                    acc[w] = p if acc[w] is None else acc[w] + p
        for w in range(W):
            a = acc[w]
            a = a + pltpu.roll(a, 64, 1)
            a = a + pltpu.roll(a, 32, 1)
            if r0 < DIL * w:
                row = lax.broadcasted_iota(jnp.int32, (RGA, 128), 0) + r0
                a = jnp.where(row >= DIL * w, a, -1e9 * LOG2E)
            lg[w, pl.ds(r0, RGA), :] = a

    def b_pv(r0):
        logits = [lg[w, pl.ds(r0, RG), :] for w in range(W)]
        m = logits[0]
        for w in range(1, W):
            m = jnp.maximum(m, logits[w])
        e = [jnp.exp2(l - m) for l in logits]
        ssum = e[0]
        for w in range(1, W):
            ssum = ssum + e[w]
        inv = pl.reciprocal(ssum, approx=True)
        inv = inv * (2.0 - ssum * inv)
        for t in range(5):
            src = 4 + t
            acc = None
            for c in range(4):
                vv = kv[src, pl.ds(HALO + r0 - DIL * c - 8, RG + 8), :]
                for w, vx in ((c, vv[8:, :]), (c + 4, vv[:RG, :])):
                    p = e[w] * vx
                    acc = p if acc is None else acc + p
            acc = acc * inv
            if t == 4:
                acc = jnp.where(lane >= 64, acc, 0.0)
            _st(ob, r0, t * 128, acc)

    def a_q(j):
        for r0 in range(0, D, AM):
            kraw[j, pl.ds(r0, AM), :] = _dot(_ld(wqT, r0, AM, 0, D), xa[:, pl.ds(j * 128, 128)])

    def a_qpost1(j, h0, nh):
        den = None
        for d in range(DH):
            rows = pl.ds(d * H + h0, nh)
            pq = _phi(kraw[j, rows, :])
            kraw[j, rows, :] = pq
            term = pq * zd[rows, :]
            den = term if den is None else den + term
        invs[j, pl.ds(h0, nh), :] = 1.0 / (den + 1e-6)

    def a_qpost2(j, h0, nh):
        inv = invs[j, pl.ds(h0, nh), :]
        for d in range(DH):
            _st(pqT, d * H + h0, j * 128, kraw[j, pl.ds(d * H + h0, nh), :] * inv)

    def out_a(j):
        for r0 in range(0, D, AM):
            _st(oaT, r0, j * 128, _dot(_ld(mT, r0, AM, 0, D), _ld(pqT, 0, D, j * 128, 128)))

    def out_apost(j, t):
        outv[pl.ds(j * 128, 128), pl.ds(t * 128, 128)] = _ld(oaT, t * 128, 128, j * 128, 128).T

    def prep_wo4():
        _st(wo4T, 0, 0, _ld(wobP, 0, DP, 0, 128).T[64:, :])

    def out_b4(j):
        _st(oaT, D, j * 128, _dot_nt(_ld(wo4T, 0, 64, 0, DP), _ld(ob, j * 128, 128, 0, DP)))

    def out_b(i, t, halves=None):
        for hh, r0 in enumerate(range(i * SB2, (i + 1) * SB2, BM)):
            if halves is not None and hh not in halves:
                continue
            obb = _dot(_ld(ob, r0, BM, 0, DP), _ld(wobP, 0, DP, t * 128, 128))
            outv[pl.ds(r0, BM), pl.ds(512 + t * 128, 128)] = obb.astype(BF16)

    def ocp(r0, nr, c0, nc, k):
        return cp(outv.at[pl.ds(r0, nr), pl.ds(c0, nc)], out_h.at[pl.ds(r0, nr), pl.ds(c0, nc)], sem_o.at[k])

    o_cp = [ocp(i * SB2, SB2, 0, 2 * D, i) for i in range(n2 - 1)]
    la_cp = ocp((n2 - 1) * SB2, SB2, 0, 640, n2)
    ol_cp = [ocp((n2 - 1) * SB2, SB2, 640 + t * 128, 128, n2 + 1 + t) for t in range(4)]

    P = functools.partial
    for c in wa_mid_cp + [xa_cp[0]]:
        c.start()

    wobP[pl.ds(8 * H, H), :] = jnp.zeros((H, DP), U32)
    for t in range(9):
        kv[t, pl.ds(0, HALO), :] = jnp.zeros((HALO, 128), F32)

    for kt in range(5):
        wa_mid_cp[kt].wait()
        if kt == 4:
            xa_cp[1].start()
        prep_wk(kt)
    xa_cp[0].wait()
    wa_lo_cp.start()
    xa_cp[2].start()


    def kpost(j):
        return [P(a_kpost, j, r0, RQ) for r0 in range(0, D, RQ)]

    side = {
        0: [],
        1: [P(prep_wq_T, kt) for kt in range(5)] + [P(prep_wq_perm, kt) for kt in range(5)],
        2: [P(prep_wb_T, kt, c0, min(c0 + 896, 1728)) for kt in range(5) for c0 in (0, 896)]
           + [P(prep_wb_perm, kt, s0, s0 + 27) for kt in range(5) for s0 in (0, 27)],
        3: [P(b_xT, j) for j in range(4)] + [P(prep_wob_shift, r0, 96) for r0 in range(0, D, 96)] + [P(prep_wob_perm, t) for t in range(5)] + [prep_wo4],
    }
    waits = {0: [xa_cp[1]], 1: [wa_lo_cp, xa_cp[2]], 2: [xa_cp[3], wb_cp], 3: xb_cp + [wob_cp, wa_hi_cp, woa_cp]}
    starts = {0: [xa_cp[3], wb_cp], 1: xb_cp, 2: [wob_cp, wa_hi_cp, woa_cp], 3: []}
    kpc = SB1 // 128
    _interleave([P(a_kT, j) for j in range(kpc)], [t for j in range(kpc - 1) for t in kpost(j)])
    for b in range(n1):
        for c in waits[b]:
            c.wait()
        for c in starts[b]:
            c.start()
        gs = [P(a_G, b, n) for n in range(5)]
        ks = [P(a_kT, (b + 1) * kpc + j) for j in range(kpc)] if b + 1 < n1 else []
        posts = kpost((b + 1) * kpc - 1) + [t for j in range(kpc - 1) for t in (kpost((b + 1) * kpc + j) if b + 1 < n1 else [])]
        if not ks:
            for t in posts:
                t()
            posts = []
        _interleave(ks + gs, posts + side[b])

    nq = SB2 // 128

    def a_chain(i):
        js = [i * nq + u for u in range(nq)]
        m = [P(a_q, j) for j in js]
        v = [P(a_qpost1, j, h0, HG) for j in js for h0 in range(0, H, HG)] + [P(a_qpost2, j, h0, HG) for j in js for h0 in range(0, H, HG)]
        m2 = [P(out_a, j) for j in js]
        v2 = [P(out_apost, j, t) for j in js for t in range(5)]
        return m, v, m2, v2

    def projs(i):
        return [P(b_xy, i * nq + u) for u in range(nq)] + [P(b_proj, i, t) for t in range(NB_T)]

    def xyposts(i):
        return [P(b_xypost, i * nq + u) for u in range(nq)]

    pj0 = projs(0)
    c1, c2 = 2, 7
    _interleave([P(a_prep_kv, c) for c in range(5)] + pj0[:c1] + [P(a_prep_M, c) for c in range(5)] + pj0[c1:c2], [a_prep_z])
    _interleave(pj0[c2:], [P(a_prep_perm, t) for t in range(5)] + xyposts(0))
    pend = []
    for i in range(n2 - 1):
        pj = projs(i + 1)
        bo = [P(out_b, i - 1, t) for t in range(5)] if i > 0 else []
        va = [P(b_logits, i * SB2 + r * RGA) for r in range(SB2 // RGA)]
        vb = [P(b_pv, i * SB2 + r * RG) for r in range(SB2 // RG)]
        xt = [P(b_xT, j) for j in range((i + 2) * nq, min((i + 3) * nq, S // 128))]
        if i >= 1:
            am, av, am2, av2 = a_chain(i - 1)
            half = [[P(out_b, i - 1, t, (h,)) for t in range(1, 5)] for h in range(2)]
            b4 = [P(out_b4, (i - 1) * nq + u) for u in range(nq)]
            na, nb = len(va) // 2, len(vb) // 2
            _interleave(am + pj[:4] + half[0] + pj[4:7], av + va[:na], lead=len(am))
            _interleave(b4 + am2 + pj[7:11] + half[1] + pj[11:],
                        av2 + va[na:] + vb[:nb] + xt + xyposts(i + 1) + vb[nb:], lead=len(b4) + len(am2))
            o_cp[i - 1].start()
            pend.append(i - 1)
        else:
            _interleave(pj, va + vb + xt + xyposts(i + 1), lead=nq)
        if i == OUT_BARRIER:
            while len(pend) > 1:
                o_cp[pend.pop(0)].wait()
    i = n2 - 1
    am, av, am2, av2 = a_chain(i - 1)
    bm, bv, bm2, bv2 = a_chain(i)
    va = [P(b_logits, i * SB2 + r * RGA) for r in range(SB2 // RGA)]
    vb = [P(b_pv, i * SB2 + r * RG) for r in range(SB2 // RG)]
    bo = [P(out_b, i - 1, t) for t in range(1, 5)] + [P(out_b4, (i - 1) * nq + u) for u in range(nq)]
    _interleave(am + bm + bo, av + bv + va, lead=len(am) + len(bm))
    _interleave(am2 + bm2, av2 + vb, lead=len(am2))
    o_cp[i - 1].start()
    pend.append(i - 1)
    for u in range(nq):
        out_b4(i * nq + u)
    for t in range(1, 5):
        for v in bv2[(t - 1) * len(bv2) // 4:t * len(bv2) // 4]:
            v()
        if t == 4:
            la_cp.start()
        out_b(i, t)
        ol_cp[t - 1].start()
    for c in [o_cp[k] for k in pend] + ol_cp + [la_cp]:
        c.wait()


@jax.jit
def pallas_concat_heads__linear_attn_block__sliding_local_dilated__prompt_kernel(
    A_x: jax.Array,
    A_wqkv: jax.Array,
    A_wo: jax.Array,
    B_x: jax.Array,
    B_wqkv: jax.Array,
    B_wo: jax.Array,
):
    n2 = S // SB2
    hbm = pl.BlockSpec(memory_space=pltpu.HBM)
    vm = pltpu.VMEM
    scratch = [
        vm((D, S), BF16),
        vm((D, S), BF16),
        vm((D, 512), BF16),
        vm((D, 640), BF16),
        vm((D, D), BF16),
        vm((D, D), BF16),
        vm((D, 3 * D), BF16),
        vm((D, D), BF16),
        vm((D // 2, D), U32),
        vm((D // 2, D), U32),
        vm((3 * D // 2, D), U32),
        vm((DP // 2, DP), U32),
        vm((D // 2, D), U32),
        vm((D, 128), F32),
        vm((5, D, 128), F32),
        vm((5, 3 * D, 128), F32),
        vm((5, D, 128), F32),
        vm((5, D, 128), F32),
        vm((D, 128), F32),
        vm((D, D), F32),
        vm((64, D), F32),
        vm((D, 128), F32),
        vm((D, D), F32),
        vm((D // 2, S), U32),
        vm((D // 2, S), U32),
        vm((S // 2, D), U32),
        vm((S // 128, D, 128), F32),
        vm((S // 128, H, 128), F32),
        vm((DP // 2, S), U32),
        vm((32, DP), U32),
        vm((5, 96, 128), U32),
        vm((S // 128, NXY, 128), F32),
        vm((5, S, 128), F32),
        vm((9, S + HALO, 128), F32),
        vm((S // 2, DP), U32),
        vm((W, S, 128), F32),
        vm((S, 2 * D), BF16),
        pltpu.SemaphoreType.DMA((2 * NXC,)),
        pltpu.SemaphoreType.DMA((11,)),
        pltpu.SemaphoreType.DMA((n2 + 6,)),
    ]
    out = pl.pallas_call(
        _kernel,
        out_shape=jax.ShapeDtypeStruct((S, 2 * D), BF16),
        in_specs=[hbm] * 6,
        out_specs=hbm,
        scratch_shapes=scratch,
        compiler_params=pltpu.CompilerParams(
            vmem_limit_bytes=100 * 1024 * 1024,
            flags={"XLA_TPU_EVENLY_DISTRIBUTE_CRITICAL_NODES": True},
        ),
    )(A_x.reshape(S, D).T, A_wqkv, A_wo, B_x.reshape(S, D).T, B_wqkv, B_wo)
    return out.reshape(1, S, 2 * D)
```
